```python
import os as _os
_os.environ.setdefault("JAX_PLATFORMS", "cpu")
import jax
import jax.numpy as jnp

def _softmax(x, axis=-1):
    return jax.nn.softmax(x, axis=axis)
def _gelu(x):
    return jax.nn.gelu(x, approximate=True)
def _silu(x):
    return jax.nn.silu(x)
def _sigmoid(x):
    return jax.nn.sigmoid(x)
def _layernorm(x, axis=-1, eps=1e-5):
    m = jnp.mean(x, axis=axis, keepdims=True)
    v = jnp.var(x, axis=axis, keepdims=True)
    return (x - m) / jnp.sqrt(v + eps)
def _scatter_add(tgt, idx, src, axis=0):
    return tgt.at[idx].add(src)
def _segment_sum(src, seg, n):
    return jax.ops.segment_sum(src, seg, n)
class _Rng:
    def __init__(self, key):
        self._k = key
    def _next(self):
        self._k, sub = jax.random.split(self._k)
        return sub
    def normal(self, shape):
        return jax.random.normal(self._next(), shape, dtype=jnp.bfloat16)
    def randint(self, lo, hi, shape):
        return jax.random.randint(self._next(), shape, lo, hi, dtype=jnp.int32)
    def uniform(self, shape, lo=0.0, hi=1.0):
        return jax.random.uniform(self._next(), shape, jnp.bfloat16, lo, hi)
    def permutation(self, n):
        return jax.random.permutation(self._next(), n)


kernel_name = 'standalone__mha_softmax__prompt'

def setup_inputs():
    _rng = _Rng(jax.random.key(int.from_bytes(__import__("os").urandom(4), "little")))
    _w = (lambda a: (lambda t: t.astype(jnp.bfloat16) if jnp.issubdtype(t.dtype, jnp.floating) else t)(jnp.asarray(a)))
    B, H, Sq, Sk, D = 1, 32, 2048, 2048, 192
    return {
        "q": _w((lambda *s: _rng.normal(s) * 0.4)(B, H, Sq, D)),
        "k": _w((lambda *s: _rng.normal(s) * 0.4)(B, H, Sk, D)),
        "v": _w((lambda *s: _rng.normal(s) * 0.05)(B, H, Sk, D)),
    }

def reference(q, k, v):
    scale = q.shape[-1] ** -0.5
    scores = jnp.einsum("bhqd,bhkd->bhqk", q, k) * scale
    p = _softmax(scores, axis=-1)
    return jnp.einsum("bhqk,bhkd->bhqd", p, v)
```

```python
import functools, math
import jax, jax.numpy as jnp
from jax import lax
from jax.experimental import pallas as pl
from jax.experimental.pallas import tpu as pltpu

LOG2E = 1.4426950408889634
f32 = jnp.float32
bf16 = jnp.bfloat16

def make(W=512, R=128, vmem=100, order='eqp', skew=0):
    tq = 2048
    def kernel(qt_ref, kt_ref, vt_ref, ot_ref, l_scr, s_scr, w_scr):
        D = qt_ref.shape[0]
        Sk = kt_ref.shape[1]
        Hf = Sk // 2
        c = (D ** -0.5) * LOG2E
        NJ = tq // W
        NC = Hf // R
        ka, kb, kc = kt_ref[0:64, 0:Hf], kt_ref[64:128, 0:Hf], kt_ref[128:192, 0:Hf]
        ka2, kb2, kc2 = kt_ref[0:64, Hf:], kt_ref[64:128, Hf:], kt_ref[128:192, Hf:]
        da = (ka.astype(f32) - ka2.astype(f32)).astype(bf16)
        dc = (kc2.astype(f32) - kc.astype(f32)).astype(bf16)
        l_scr[0] = jnp.concatenate([da, kb], axis=0).T
        l_scr[1] = jnp.concatenate([kb2, dc], axis=0).T
        l_scr[2] = jnp.concatenate([kc, ka2], axis=0).T
        for j in range(NJ):
            qs = (qt_ref[:, j*W:(j+1)*W].astype(f32) * c).astype(bf16)
            w_scr[j, 0:192, :] = qs
            w_scr[j, 192:256, :] = qs[0:64, :]
        def qk_chunk(j, b, cc, mpart):
            r = slice(cc*R, (cc+1)*R)
            w1 = w_scr[j, 0:128, :]; w2 = w_scr[j, 64:192, :]; w3 = w_scr[j, 128:256, :]
            t3 = jnp.dot(l_scr[2, r, :], w3, preferred_element_type=f32)
            s1 = jnp.dot(l_scr[0, r, :], w1, preferred_element_type=f32) + t3
            s2 = jnp.dot(l_scr[1, r, :], w2, preferred_element_type=f32) + t3
            s_scr[b, cc*2*R:cc*2*R+R, :] = s1
            s_scr[b, cc*2*R+R:(cc+1)*2*R, :] = s2
            mx = jnp.max(jnp.maximum(s1, s2).reshape(R//8, 8, W), axis=0)
            return mx if mpart is None else jnp.maximum(mpart, mx)
        def exp_chunk(b, cc, m, lpart):
            p1 = jnp.exp2(s_scr[b, cc*2*R:cc*2*R+R, :] - m)
            p2 = jnp.exp2(s_scr[b, cc*2*R+R:(cc+1)*2*R, :] - m)
            ls = jnp.sum((p1 + p2).reshape(R//8, 8, W), axis=0)
            return (ls if lpart is None else lpart + ls), p1.astype(bf16), p2.astype(bf16)
        def pv_chunk(cc, p1, p2, acc):
            o1 = jnp.dot(vt_ref[:, cc*R:(cc+1)*R], p1, preferred_element_type=f32)
            o2 = jnp.dot(vt_ref[:, Hf+cc*R:Hf+(cc+1)*R], p2, preferred_element_type=f32)
            o = o1 + o2
            return (o if acc is None else acc + o)
        def tile(j, mpart_in, do_qk):
            b = j % 2
            m = jnp.max(mpart_in, axis=0, keepdims=True)
            mpart = None; lpart = None; acc = None
            for cc in range(NC):
                lpart, p1, p2 = exp_chunk(b, cc, m, lpart)
                if do_qk:
                    mpart = qk_chunk(j+1, 1-b, cc, mpart)
                acc = pv_chunk(cc, p1, p2, acc)
            l = jnp.sum(lpart, axis=0, keepdims=True)
            o = (acc * (1.0 / l)).astype(ot_ref.dtype)
            if isinstance(j, int):
                ot_ref[:, j*W:(j+1)*W] = o
            else:
                ot_ref[:, pl.ds(pl.multiple_of(j*W, W), W)] = o
            return mpart
        mpart = None
        for cc in range(NC):
            mpart = qk_chunk(0, 0, cc, mpart)
        mpart = lax.fori_loop(0, NJ-1, lambda j, mp: tile(j, mp, True), mpart)
        tile(NJ-1, mpart, False)

    def fn(q, k, v):
        B, H, Sq, D = q.shape
        Sk = k.shape[2]
        qt = jnp.swapaxes(q, -1, -2).reshape(B*H, D, Sq)
        kt = jnp.swapaxes(k, -1, -2).reshape(B*H, D, Sk)
        vt = jnp.swapaxes(v, -1, -2).reshape(B*H, D, Sk)
        ot = pl.pallas_call(
            kernel,
            grid=(B*H,),
            in_specs=[
                pl.BlockSpec((None, D, tq), lambda h: (h, 0, 0)),
                pl.BlockSpec((None, D, Sk), lambda h: (h, 0, 0)),
                pl.BlockSpec((None, D, Sk), lambda h: (h, 0, 0)),
            ],
            out_specs=pl.BlockSpec((None, D, tq), lambda h: (h, 0, 0)),
            out_shape=jax.ShapeDtypeStruct((B*H, D, Sq), q.dtype),
            scratch_shapes=[pltpu.VMEM((3, Sk // 2, 128), jnp.bfloat16),
                            pltpu.VMEM((2, Sk, W), f32),
                            pltpu.VMEM((tq // W, 256, W), bf16)],
            compiler_params=pltpu.CompilerParams(
                dimension_semantics=("arbitrary",),
                vmem_limit_bytes=vmem * 1024 * 1024),
        )(qt, kt, vt)
        return jnp.swapaxes(ot.reshape(B, H, D, Sq), -1, -2)
    return fn


_FN = make(W=256, R=128)

@jax.jit
def pallas_standalone__mha_softmax__prompt_kernel(q, k, v):
    return _FN(q, k, v)
```

```python
import jax
import jax.numpy as jnp
from jax import lax
from jax.experimental import pallas as pl
from jax.experimental.pallas import tpu as pltpu

LOG2E = 1.4426950408889634
f32 = jnp.float32
bf16 = jnp.bfloat16


def make(W=256, R=128, vmem=64, gate=2, egate=3, hv=True, hl=True, hq=True, nobc=False, rot=2,
         ksp=(4,), qmerge=False, pro_start=1, mmode='pair'):
    def kernel(q_hbm, k_hbm, v_hbm, o_hbm, qbuf, kbuf, vbuf, obuf, l_scr, s0, s1, m_scr, sem):
        BH, D, Sq = q_hbm.shape
        Sk = k_hbm.shape[2]
        G = D // 3
        c = (D ** -0.5) * LOG2E
        NJ = Sq // W
        NC = Sk // (2 * R)
        NI = BH - 1
        s_bufs = (s0, s1)
        phase = pl.program_id(0)
        z = phase // 3

        def cp_k(h, p): return pltpu.make_async_copy(k_hbm.at[h], kbuf.at[p], sem.at[0])
        def cp_q(h, p): return pltpu.make_async_copy(q_hbm.at[h], qbuf.at[p], sem.at[1])
        def cp_v(h, p): return pltpu.make_async_copy(v_hbm.at[h], vbuf.at[p], sem.at[2])
        def cp_o(h, p): return pltpu.make_async_copy(obuf.at[p], o_hbm.at[h], sem.at[3])
        def cp_cols(src, dst, a, n, s):
            return pltpu.make_async_copy(src.at[:, pl.ds(a, n)], dst.at[:, pl.ds(a, n)], sem.at[s])

        cache = {}
        def cached(on, key, f):
            if key in cache: return cache[key]
            if not on: return f()
            cache[key] = f()
            return cache[key]

        def prep(k_ref, cc, gen):
            lo = slice(2*R*cc, 2*R*cc + R); hi = slice(2*R*cc + R, 2*R*(cc + 1))
            ka, kb, kc = k_ref[0:G, lo], k_ref[G:2*G, lo], k_ref[2*G:3*G, lo]
            ka2, kb2, kc2 = k_ref[0:G, hi], k_ref[G:2*G, hi], k_ref[2*G:3*G, hi]
            da = (ka.astype(f32) - ka2.astype(f32)).astype(bf16)
            dc = (kc2.astype(f32) - kc.astype(f32)).astype(bf16)
            for i, parts in ((2, [kc, ka2]), (0, [da, kb]), (1, [kb2, dc])):
                t = jnp.concatenate(parts, axis=0).T
                l_scr[i, cc*R:(cc+1)*R, :] = t
                cache[('l', gen, i, cc)] = t

        def qk_chunk(q_ref, j, cc, mpart, gen):
            sl = slice(j*W, (j+1)*W)
            qa = cached(hq, ('qa', gen, j), lambda: q_ref[0:G, sl])
            qb = cached(hq, ('qb', gen, j), lambda: q_ref[G:2*G, sl])
            qc = cached(hq, ('qc', gen, j), lambda: q_ref[2*G:3*G, sl])
            ws = (jnp.concatenate([qa, qb], axis=0), jnp.concatenate([qb, qc], axis=0), jnp.concatenate([qc, qa], axis=0))
            r = {}
            for i in (2, 0, 1):
                r[i] = jnp.dot(cached(hl, ('l', gen, i, cc), lambda: l_scr[i, cc*R:(cc+1)*R, :]), ws[i], preferred_element_type=f32)
            s1_ = r[0] + r[2]
            s2_ = r[1] + r[2]
            s_bufs[j % 2][z, cc*2*R:cc*2*R+R, :] = s1_
            s_bufs[j % 2][z, cc*2*R+R:(cc+1)*2*R, :] = s2_
            if mmode == 'pair':
                mx = jnp.max(jnp.maximum(s1_, s2_).reshape(R//8, 8, W), axis=0)
            else:
                mx = jnp.maximum(jnp.max(s1_.reshape(R//8, 8, W), axis=0), jnp.max(s2_.reshape(R//8, 8, W), axis=0))
            return mx if mpart is None else jnp.maximum(mpart, mx)

        def exp_chunk(j, cc, m, ls):
            ps = []
            for a in (cc*2*R, cc*2*R + R):
                x = (s_bufs[j % 2][0, a:a+R, :].reshape(R//8, 8, W) - m[None]) * c
                ps.append(jnp.exp2(x.reshape(R, W)))
            for p in ps:
                for i in reversed(range(R // 16)):
                    x = p[i*16:i*16+8] + p[i*16+8:i*16+16]
                    ls = x if ls is None else ls + x
            return ls, ps[0].astype(bf16), ps[1].astype(bf16)

        def pv_chunk(vt_ref, vgen, cc, p1, p2, acc):
            v1 = cached(hv, ('v1', vgen, cc), lambda: vt_ref[:, cc*2*R:cc*2*R+R])
            v2 = cached(hv, ('v2', vgen, cc), lambda: vt_ref[:, cc*2*R+R:(cc+1)*2*R])
            o1 = jnp.dot(v1, p1, preferred_element_type=f32)
            o2 = jnp.dot(v2, p2, preferred_element_type=f32)
            return (o1 if acc is None else acc + o1) + o2

        def step(j, mpart_in, pv, vgen, pq, gen, with_prep=False):
            m = jnp.broadcast_to(jnp.max(mpart_in, axis=0, keepdims=True), (8, W))
            hist = []
            mpart = None; lpart = None; acc = None
            if with_prep:
                for cc in range(NC): prep(kbuf.at[pq], cc, gen)
            g = gate if pq is not None else egate
            for cc in range(NC):
                mg = m
                if g and cc >= g:
                    mg = jnp.where(z > 0, hist[cc - g], m)
                lpart, p1, p2 = exp_chunk(j, cc, mg, lpart)
                if pq is not None:
                    mpart = qk_chunk(qbuf.at[pq], (j + 1) % NJ, cc, mpart, gen)
                acc = pv_chunk(vbuf.at[pv], vgen, cc, p1, p2, acc)
                hist.append(mpart if pq is not None else acc[0:8])
            l = jnp.sum(lpart, axis=0, keepdims=True)
            obuf[pv, :, j*W:(j+1)*W] = (acc * (1.0 / l)).astype(obuf.dtype)
            return mpart

        @pl.when(phase == 0)
        def _():
            bounds = (0,) + tuple(ksp) + (NC,)
            cks = [cp_cols(k_hbm.at[0], kbuf.at[1], 2*R*bounds[i], 2*R*(bounds[i+1]-bounds[i]), 7 + i) for i in range(len(bounds) - 1)]
            cq0 = cp_cols(q_hbm.at[0], qbuf.at[1], 0, 2 * W, 4)
            cq1 = cp_cols(q_hbm.at[0], qbuf.at[1], 2 * W, Sq - 2 * W, 5)
            cv = pltpu.make_async_copy(v_hbm.at[0], vbuf.at[1], sem.at[6])
            cks[0].start(); cq0.start()
            for ck in cks[1:]: ck.start()
            cv.start(); cq1.start()
            mp = None
            cq0.wait()
            for cc in range(NC):
                if cc in bounds: cks[bounds.index(cc)].wait()
                prep(kbuf.at[1], cc, 'p0')
                mp = qk_chunk(qbuf.at[1], 0, cc, mp, 'p0')
            cv.wait()
            if qmerge: cq1.wait()
            h1 = min(1, BH - 1)
            for j in range(NJ - rot):
                if j == 1 and not qmerge: cq1.wait()
                if j == pro_start:
                    cp_k(h1, 0).start(); cp_q(h1, 0).start(); cp_v(h1, 0).start()
                tag = 'p2' if (j > 0 or qmerge) else 'p1'
                mp = step(j, mp, 1, tag, 1, tag)
            m_scr[...] = mp
            cp_k(h1, 0).wait(); cp_q(h1, 0).wait(); cp_v(h1, 0).wait()

        @pl.when(phase == 1)
        def _():
            def body(it, mp):
                p = jnp.bitwise_and(it, 1)
                pp = 1 - p
                h2 = jnp.minimum(it + 2, BH - 1)
                cp_k(h2, pp).start()
                for j in range(NJ - rot, NJ - 1):
                    mp = step(j, mp, pp, 'b0', pp, 'b0')
                mp = step(NJ - 1, mp, pp, 'b0', p, 'b1', with_prep=True)
                cp_q(h2, pp).start()
                cp_v(h2, pp).start()
                cp_o(it, pp).start()
                for j in range(NJ - rot):
                    mp = step(j, mp, p, 'b1', p, 'b1')
                cp_k(h2, pp).wait(); cp_q(h2, pp).wait(); cp_v(h2, pp).wait()
                cp_o(it, pp).wait()
                return mp
            m_scr[...] = lax.fori_loop(0, NI, body, m_scr[...])

        @pl.when(phase == 2)
        def _():
            pp = 1 - NI % 2
            a = (NJ - 1) * W
            co0 = cp_cols(obuf.at[pp], o_hbm.at[BH - 1], 0, a, 4)
            co1 = cp_cols(obuf.at[pp], o_hbm.at[BH - 1], a, W, 5)
            mp = m_scr[...]
            for j in range(NJ - rot, NJ - 1):
                mp = step(j, mp, pp, 'e', pp, 'e')
            co0.start()
            step(NJ - 1, mp, pp, 'e', None, None)
            co1.start()
            co0.wait(); co1.wait()

    def fn(q, k, v):
        B, H, Sq, D = q.shape
        Sk = k.shape[2]
        BH = B * H
        qt = jnp.swapaxes(q, -1, -2).reshape(BH, D, Sq)
        kt = jnp.swapaxes(k, -1, -2).reshape(BH, D, Sk)
        vt = jnp.swapaxes(v, -1, -2).reshape(BH, D, Sk)
        ot = pl.pallas_call(
            kernel,
            grid=(3,),
            in_specs=[pl.BlockSpec(memory_space=pl.ANY)] * 3,
            out_specs=pl.BlockSpec(memory_space=pl.ANY),
            out_shape=jax.ShapeDtypeStruct((BH, D, Sq), q.dtype),
            scratch_shapes=[pltpu.VMEM((2, D, Sq), bf16), pltpu.VMEM((2, D, Sk), bf16),
                            pltpu.VMEM((2, D, Sk), bf16), pltpu.VMEM((2, D, Sq), bf16),
                            pltpu.VMEM((3, Sk // 2, 128), bf16),
                            pltpu.VMEM((2, Sk, W), f32), pltpu.VMEM((2, Sk, W), f32),
                            pltpu.VMEM((8, W), f32),
                            pltpu.SemaphoreType.DMA((8 + len(ksp),))],
            compiler_params=pltpu.CompilerParams(
                dimension_semantics=("arbitrary",),
                vmem_limit_bytes=vmem * 1024 * 1024, disable_bounds_checks=nobc),
        )(qt, kt, vt)
        return jnp.swapaxes(ot.reshape(B, H, D, Sq), -1, -2)
    return fn


_FN = make()

@jax.jit
def pallas_standalone__mha_softmax__prompt_kernel(q, k, v):
    return _FN(q, k, v)
```

```python
import jax
import jax.numpy as jnp
from jax import lax
from jax.experimental import pallas as pl
from jax.experimental.pallas import tpu as pltpu

_LOG2E = 1.4426950408889634
_F32 = jnp.float32
_BF16 = jnp.bfloat16

_W = 256
_R = 128
_ROT = 2
_K_FIRST = 2
_GATE = 2
_GATE_PV = 5


def _attn_kernel(q_hbm, k_hbm, v_hbm, o_hbm,
                 qbuf, kbuf, vbuf, obuf, l_scr, s0, s1, m_scr, sem):
    W, R = _W, _R
    BH, D, Sq = q_hbm.shape
    Sk = k_hbm.shape[2]
    G = D // 3
    c = (D ** -0.5) * _LOG2E
    NJ = Sq // W
    NC = Sk // (2 * R)
    NI = BH - 1
    s_bufs = (s0, s1)
    phase = pl.program_id(0)
    z = phase // 3

    def cp_k(h, p):
        return pltpu.make_async_copy(k_hbm.at[h], kbuf.at[p], sem.at[0])

    def cp_q(h, p):
        return pltpu.make_async_copy(q_hbm.at[h], qbuf.at[p], sem.at[1])

    def cp_v(h, p):
        return pltpu.make_async_copy(v_hbm.at[h], vbuf.at[p], sem.at[2])

    def cp_o(h, p):
        return pltpu.make_async_copy(obuf.at[p], o_hbm.at[h], sem.at[3])

    def cp_cols(src, dst, a, n, s):
        return pltpu.make_async_copy(
            src.at[:, pl.ds(a, n)], dst.at[:, pl.ds(a, n)], sem.at[s])

    cache = {}

    def cached(key, load):
        if key not in cache:
            cache[key] = load()
        return cache[key]

    def prep(k_ref, cc, gen):
        lo = slice(2 * R * cc, 2 * R * cc + R)
        hi = slice(2 * R * cc + R, 2 * R * (cc + 1))
        ka, kb, kc = k_ref[0:G, lo], k_ref[G:2 * G, lo], k_ref[2 * G:D, lo]
        ka2, kb2, kc2 = k_ref[0:G, hi], k_ref[G:2 * G, hi], k_ref[2 * G:D, hi]
        da = (ka.astype(_F32) - ka2.astype(_F32)).astype(_BF16)
        dc = (kc2.astype(_F32) - kc.astype(_F32)).astype(_BF16)
        for i, parts in ((2, [kc, ka2]), (0, [da, kb]), (1, [kb2, dc])):
            t = jnp.concatenate(parts, axis=0).T
            l_scr[i, cc * R:(cc + 1) * R, :] = t
            cache[("l", gen, i, cc)] = t

    def qk_chunk(q_ref, j, cc, mpart, gen):
        sl = slice(j * W, (j + 1) * W)
        qa = cached(("qa", gen, j), lambda: q_ref[0:G, sl])
        qb = cached(("qb", gen, j), lambda: q_ref[G:2 * G, sl])
        qc = cached(("qc", gen, j), lambda: q_ref[2 * G:D, sl])
        ws = (jnp.concatenate([qa, qb], axis=0),
              jnp.concatenate([qb, qc], axis=0),
              jnp.concatenate([qc, qa], axis=0))
        r = {}
        for i in (2, 0, 1):
            lhs = cached(("l", gen, i, cc),
                         lambda: l_scr[i, cc * R:(cc + 1) * R, :])
            r[i] = jnp.dot(lhs, ws[i], preferred_element_type=_F32)
        sa = r[0] + r[2]
        sb = r[1] + r[2]
        s_bufs[j % 2][z, cc * 2 * R:cc * 2 * R + R, :] = sa
        s_bufs[j % 2][z, cc * 2 * R + R:(cc + 1) * 2 * R, :] = sb
        mx = jnp.maximum(jnp.max(sa.reshape(R // 8, 8, W), axis=0),
                         jnp.max(sb.reshape(R // 8, 8, W), axis=0))
        return mx if mpart is None else jnp.maximum(mpart, mx)

    def exp_chunk(j, cc, m, ls):
        ps = []
        for a in (cc * 2 * R, cc * 2 * R + R):
            x = (s_bufs[j % 2][0, a:a + R, :].reshape(R // 8, 8, W) - m[None]) * c
            ps.append(jnp.exp2(x.reshape(R, W)))
        for p in ps:
            for i in reversed(range(R // 16)):
                x = p[i * 16:i * 16 + 8] + p[i * 16 + 8:i * 16 + 16]
                ls = x if ls is None else ls + x
        return ls, ps[0].astype(_BF16), ps[1].astype(_BF16)

    def pv_chunk(v_ref, cc, p1, p2, acc):
        o1 = jnp.dot(v_ref[:, cc * 2 * R:cc * 2 * R + R], p1,
                     preferred_element_type=_F32)
        o2 = jnp.dot(v_ref[:, cc * 2 * R + R:(cc + 1) * 2 * R], p2,
                     preferred_element_type=_F32)
        return (o1 if acc is None else acc + o1) + o2

    def step(j, mpart_in, pv, pq, gen, with_prep=False):
        m = jnp.broadcast_to(jnp.max(mpart_in, axis=0, keepdims=True), (8, W))
        hist = []
        mpart = lpart = acc = None
        if with_prep:
            for cc in range(NC):
                prep(kbuf.at[pq], cc, gen)
        g = _GATE if pq is not None else _GATE_PV
        for cc in range(NC):
            mg = m if cc < g else jnp.where(z > 0, hist[cc - g], m)
            lpart, p1, p2 = exp_chunk(j, cc, mg, lpart)
            if pq is not None:
                mpart = qk_chunk(qbuf.at[pq], (j + 1) % NJ, cc, mpart, gen)
            acc = pv_chunk(vbuf.at[pv], cc, p1, p2, acc)
            hist.append(mpart if pq is not None else acc[0:8])
        l = jnp.sum(lpart, axis=0, keepdims=True)
        obuf[pv, :, j * W:(j + 1) * W] = (acc * (1.0 / l)).astype(obuf.dtype)
        return mpart

    @pl.when(phase == 0)
    def _():
        cache.clear()
        n0 = 2 * R * _K_FIRST
        ck0 = cp_cols(k_hbm.at[0], kbuf.at[1], 0, n0, 7)
        ck1 = cp_cols(k_hbm.at[0], kbuf.at[1], n0, Sk - n0, 8)
        cq0 = cp_cols(q_hbm.at[0], qbuf.at[1], 0, 2 * W, 4)
        cq1 = cp_cols(q_hbm.at[0], qbuf.at[1], 2 * W, Sq - 2 * W, 5)
        cv = pltpu.make_async_copy(v_hbm.at[0], vbuf.at[1], sem.at[6])
        for cp in (ck0, cq0, ck1, cv, cq1):
            cp.start()
        cq0.wait()
        ck0.wait()
        mps = [None, None]
        for cc in range(NC):
            if cc == _K_FIRST:
                ck1.wait()
            prep(kbuf.at[1], cc, "p0")
            for t in (0, 1):
                mps[t] = qk_chunk(qbuf.at[1], t, cc, mps[t], "p0")
        cv.wait()
        cq1.wait()
        nxt = (cp_k(1, 0), cp_q(1, 0), cp_v(1, 0))
        for cp in nxt:
            cp.start()
        step(0, mps[0], 1, None, None)
        mp = mps[1]
        for j in range(1, NJ - _ROT):
            mp = step(j, mp, 1, 1, "p1")
        m_scr[...] = mp
        for cp in nxt:
            cp.wait()

    @pl.when(phase == 1)
    def _():
        def body(it, mp):
            cache.clear()
            p = jnp.bitwise_and(it, 1)
            pp = 1 - p
            h2 = jnp.minimum(it + 2, BH - 1)
            ck, cq, cv, co = cp_k(h2, pp), cp_q(h2, pp), cp_v(h2, pp), cp_o(it, pp)
            ck.start()
            for j in range(NJ - _ROT, NJ - 1):
                mp = step(j, mp, pp, pp, "b0")
            mp = step(NJ - 1, mp, pp, p, "b1", with_prep=True)
            cq.start()
            cv.start()
            co.start()
            for j in range(NJ - _ROT):
                mp = step(j, mp, p, p, "b1")
            for cp in (ck, cq, cv, co):
                cp.wait()
            return mp

        m_scr[...] = lax.fori_loop(0, NI, body, m_scr[...])

    @pl.when(phase == 2)
    def _():
        cache.clear()
        pp = 1 - NI % 2
        a = (NJ - 1) * W
        co0 = cp_cols(obuf.at[pp], o_hbm.at[BH - 1], 0, a, 4)
        co1 = cp_cols(obuf.at[pp], o_hbm.at[BH - 1], a, W, 5)
        mp = m_scr[...]
        for j in range(NJ - _ROT, NJ - 1):
            mp = step(j, mp, pp, pp, "e")
        co0.start()
        step(NJ - 1, mp, pp, None, None)
        co1.start()
        co0.wait()
        co1.wait()


@jax.jit
def pallas_standalone__mha_softmax__prompt_kernel(
    q: jax.Array,
    k: jax.Array,
    v: jax.Array,
):
    B, H, Sq, D = q.shape
    Sk = k.shape[2]
    BH = B * H
    assert D == 192 and BH >= 2
    assert Sq % (2 * _W) == 0 and Sq // _W >= 2 + _ROT
    assert Sk % (2 * _R) == 0 and Sk // (2 * _R) > max(_K_FIRST, _GATE_PV)

    qt = jnp.swapaxes(q, -1, -2).reshape(BH, D, Sq)
    kt = jnp.swapaxes(k, -1, -2).reshape(BH, D, Sk)
    vt = jnp.swapaxes(v, -1, -2).reshape(BH, D, Sk)
    ot = pl.pallas_call(
        _attn_kernel,
        grid=(3,),
        in_specs=[pl.BlockSpec(memory_space=pl.ANY)] * 3,
        out_specs=pl.BlockSpec(memory_space=pl.ANY),
        out_shape=jax.ShapeDtypeStruct((BH, D, Sq), q.dtype),
        scratch_shapes=[
            pltpu.VMEM((2, D, Sq), _BF16),
            pltpu.VMEM((2, D, Sk), _BF16),
            pltpu.VMEM((2, D, Sk), _BF16),
            pltpu.VMEM((2, D, Sq), _BF16),
            pltpu.VMEM((3, Sk // 2, 128), _BF16),
            pltpu.VMEM((2, Sk, _W), _F32),
            pltpu.VMEM((2, Sk, _W), _F32),
            pltpu.VMEM((8, _W), _F32),
            pltpu.SemaphoreType.DMA((9,)),
        ],
        compiler_params=pltpu.CompilerParams(
            dimension_semantics=("arbitrary",),
            vmem_limit_bytes=64 * 1024 * 1024,
        ),
    )(qt, kt, vt)
    return jnp.swapaxes(ot.reshape(B, H, D, Sq), -1, -2)
```
